```python
import os as _os
_os.environ.setdefault("JAX_PLATFORMS", "cpu")
import jax
import jax.numpy as jnp

def _softmax(x, axis=-1):
    return jax.nn.softmax(x, axis=axis)
def _gelu(x):
    return jax.nn.gelu(x, approximate=True)
def _silu(x):
    return jax.nn.silu(x)
def _sigmoid(x):
    return jax.nn.sigmoid(x)
def _layernorm(x, axis=-1, eps=1e-5):
    m = jnp.mean(x, axis=axis, keepdims=True)
    v = jnp.var(x, axis=axis, keepdims=True)
    return (x - m) / jnp.sqrt(v + eps)
def _scatter_add(tgt, idx, src, axis=0):
    return tgt.at[idx].add(src)
def _segment_sum(src, seg, n):
    return jax.ops.segment_sum(src, seg, n)
class _Rng:
    def __init__(self, key):
        self._k = key
    def _next(self):
        self._k, sub = jax.random.split(self._k)
        return sub
    def normal(self, shape):
        return jax.random.normal(self._next(), shape, dtype=jnp.bfloat16)
    def randint(self, lo, hi, shape):
        return jax.random.randint(self._next(), shape, lo, hi, dtype=jnp.int32)
    def uniform(self, shape, lo=0.0, hi=1.0):
        return jax.random.uniform(self._next(), shape, jnp.bfloat16, lo, hi)
    def permutation(self, n):
        return jax.random.permutation(self._next(), n)


kernel_name = 'recurrent_scan__ssm_conv_s4__mixer_s_mlp__prompt'

def setup_inputs():
    _rng = _Rng(jax.random.key(int.from_bytes(__import__("os").urandom(4), "little")))
    _w = (lambda a: (lambda t: t.astype(jnp.bfloat16) if jnp.issubdtype(t.dtype, jnp.floating) else t)(jnp.asarray(a)))
    def _A_setup():
        B, L, D, N = 1, 2048, 512, 128
        A_re = -jnp.exp((lambda *s: _rng.normal(s) * 0.1)(D, N))
        A_im = jnp.pi * (lambda *s: _rng.normal(s) * 0.1)(D, N)
        B_re = (lambda *s: _rng.normal(s) * 0.1)(D, N)
        B_im = (lambda *s: _rng.normal(s) * 0.1)(D, N)
        C_re = (lambda *s: _rng.normal(s) * 0.1)(D, N)
        C_im = (lambda *s: _rng.normal(s) * 0.1)(D, N)
        log_dt = (lambda *s: _rng.normal(s) * 0.1)(D) * 0.5 - 4.0
        Dskip = (lambda *s: _rng.normal(s) * 0.05)(D)
        return {
            "u": _w((lambda *s: _rng.normal(s) * 0.05)(B, L, D)),
            "A_re": _w(A_re),
            "A_im": _w(A_im),
            "B_re": _w(B_re),
            "B_im": _w(B_im),
            "C_re": _w(C_re),
            "C_im": _w(C_im),
            "log_dt": _w(log_dt),
            "Dskip": _w(Dskip),
        }
    _A_in = _A_setup()

    def _B_setup():
        B, S, D, F = 1, 2048, 512, 1376
        return {
            "x":  _w((lambda *s: _rng.normal(s) * 0.05)(B, S, D)),
            "w1": _w((lambda *s: _rng.normal(s) * 0.8)(D, D) * (D ** -0.5)),
            "w2": _w((lambda *s: _rng.normal(s) * 0.8)(D, D) * (D ** -0.5)),
            "w3": _w((lambda *s: _rng.normal(s) * 0.8)(D, F) * (D ** -0.5)),
            "w4": _w((lambda *s: _rng.normal(s) * 0.8)(F, D) * (F ** -0.5)),
        }
    _B_in = _B_setup()

    return {
        "A_u": _A_in["u"],
        "A_A_re": _A_in["A_re"],
        "A_A_im": _A_in["A_im"],
        "A_B_re": _A_in["B_re"],
        "A_B_im": _A_in["B_im"],
        "A_C_re": _A_in["C_re"],
        "A_C_im": _A_in["C_im"],
        "A_log_dt": _A_in["log_dt"],
        "A_Dskip": _A_in["Dskip"],
        "B_x": _B_in["x"],
        "B_w1": _B_in["w1"],
        "B_w2": _B_in["w2"],
        "B_w3": _B_in["w3"],
        "B_w4": _B_in["w4"],
    }

def reference(A_u, A_A_re, A_A_im, A_B_re, A_B_im, A_C_re, A_C_im, A_log_dt, A_Dskip, B_x, B_w1, B_w2, B_w3, B_w4):
    def _A_ref(u, A_re, A_im, B_re, B_im, C_re, C_im, log_dt, Dskip):
        Bsz, L, D = u.shape
        dt = jnp.exp(log_dt)[:, None]
        A = A_re + 1j * A_im
        Bc = B_re + 1j * B_im
        Cc = C_re + 1j * C_im
        logdA = dt * A
        dB = dt * Bc
        l = (lambda x, dt: x.astype(dt))(jnp.arange(L), A_re.dtype)
        P = jnp.exp(logdA[:, :, None] * l[None, None, :])
        K = jnp.einsum("dn,dnl,dn->dl", Cc, P, dB).real
        L2 = 2 * L
        Kp = jnp.pad(K, ((0, 0), (0, L)))
        up = (lambda x, *d: x.transpose(*d))(u, 0, 2, 1)
        up = jnp.pad(up, ((0, 0), (0, 0), (0, L)))
        Kf = (lambda x, axes=(-2,-1): jnp.fft.rfft2(x.astype(jnp.float32), axes=axes))(Kp[:, None, :], axes=(-2, -1))
        Uf = (lambda x, axes=(-2,-1): jnp.fft.rfft2(x.astype(jnp.float32), axes=axes))(up[:, :, None, :], axes=(-2, -1))
        Yf = Uf * Kf[None, :, :, :]
        y = (lambda x, s, axes=(-2,-1): jnp.fft.irfft2(x, s=s, axes=axes).astype(jnp.bfloat16))(Yf, (1, L2), axes=(-2, -1))[:, :, 0, :L]
        y = (lambda x, *d: x.transpose(*d))(y, 0, 2, 1) + u * Dskip[None, None, :]
        return y

    def _B_ref(x, w1, w2, w3, w4):
        B, S, D = x.shape
        h = _gelu(_layernorm(x, axis=-1) @ w1)
        c = D // 4
        g0 = jnp.pad(h[:, :, 0*c:1*c], ((0, 0), (1, 0), (0, 0)))[:, :S, :]
        g1 = jnp.pad(h[:, :, 1*c:2*c], ((0, 0), (0, 1), (0, 0)))[:, 1:, :]
        g2 = jnp.pad(h[:, :, 2*c:3*c], ((0, 0), (2, 0), (0, 0)))[:, :S, :]
        g3 = jnp.pad(h[:, :, 3*c:   ], ((0, 0), (0, 2), (0, 0)))[:, 2:, :]
        hs = jnp.concatenate([g0, g1, g2, g3], axis=-1) @ w2
        x1 = x + hs
        h2 = _gelu(_layernorm(x1, axis=-1) @ w3) @ w4
        return x1 + h2

    x = A_u
    xn = _layernorm(x, axis=-1)
    s = _A_ref(xn, A_A_re, A_A_im, A_B_re, A_B_im, A_C_re, A_C_im, A_log_dt, A_Dskip)
    g = _silu(_B_ref(xn, B_w1, B_w2, B_w3, B_w4))
    return x + s * g
```

```python
import numpy as np
import jax
import jax.numpy as jnp
from jax import lax
import jax.experimental.pallas as pl
import jax.experimental.pallas.tpu as pltpu

L, D, N, F = 2048, 512, 128, 1376
Q = 128
NC = L // Q
BF = jnp.bfloat16
F32 = jnp.float32
TILE_OFFS = [[1, 3, 5, 7], [2, 4, 6, 8], [258, 260, 262, 264], [516, 520, 772, 776],
             [1032, 1288], [1544, 1800]]
PIECES = [(0, 0, None), (0, 1, None), (1, 0, None), (1, 1, None), (2, 2, (1, 2)), (3, 2, None),
          (4, 3, (2, 126)), (5, 3, None), (6, 3, None), (7, 3, None), (8, 4, (3, 2)), (9, 4, None),
          (10, 4, None), (11, 4, None), (12, 5, (4, 124)), (13, 5, None), (14, 5, None), (15, 5, None)]


def _lane_vals(t):
    v = np.full(128, -1, np.int64)
    for i, off in enumerate(TILE_OFFS[t]):
        for j in range(32):
            v[(4 * j + i + 3 + 4 * (t % 2)) % 128] = off + 8 * j
    return v


def _consts():
    k = np.concatenate([np.arange(0, Q, 2), np.arange(1, Q, 2)])
    w = 2 * np.pi * (k + 0.5) / (2 * Q)
    def fm(p):
        a = w[:, None] * p[None, :]
        return np.concatenate([np.cos(a), -np.sin(a)], 0)
    fwd = fm(np.arange(Q))
    inv = fwd.T / Q
    lb = np.arange(L).astype(np.float32).astype(BF).astype(np.int64)
    fk = np.zeros((len(PIECES), 2 * Q, 128))
    used = set()
    for p, (m, t, t2) in enumerate(PIECES):
        vals = _lane_vals(t)
        if t2 is not None:
            vals[t2[1]] = _lane_vals(t2[0])[(t2[1] + 4) % 128]
        for l in range(Q * m + 1, min(Q * m + Q + 1, L)):
            idx = np.nonzero(vals == lb[l])[0]
            if len(idx):
                fk[p, :, idx[0]] += fm(np.array([l - Q * m]))[:, 0]
                assert l not in used
                used.add(l)
    assert len(used) == L - 1
    return fwd.astype(BF), inv.astype(BF), fk.astype(BF)


FWD, INV, FK = _consts()


def cmul(a, b):
    return a[0] * b[0] - a[1] * b[1], a[0] * b[1] + a[1] * b[0]


def csq(a):
    x = a[0] * a[1]
    return a[0] * a[0] - a[1] * a[1], x + x


def csel(m, a, b):
    return jnp.where(m, a[0], b[0]), jnp.where(m, a[1], b[1])


def ln(x):
    m = jnp.mean(x, axis=-1, keepdims=True)
    d = x - m
    v = jnp.mean(d * d, axis=-1, keepdims=True)
    return d * lax.rsqrt(v + 1e-5)


def gelu(x):
    c = 0.7978845608028654
    return (0.5 * x) * (1.0 + jnp.tanh(x * (c + (c * 0.044715) * (x * x))))


def dot(a, b):
    return jnp.dot(a, b, preferred_element_type=F32)


def dot_nt(a, b):
    return lax.dot_general(a, b, (((1,), (1,)), ((), ())), preferred_element_type=F32)


GS = (0.7978845608028654 * 0.044715) ** (1.0 / 3.0)
GA = 0.7978845608028654 / GS
GO = 0.5 / GS


def gelu_s(v):
    return v + v * jnp.tanh(v * (GA + v * v))


def ln_s(x, scale):
    m = jnp.mean(x, axis=-1, keepdims=True)
    d = x - m
    v = jnp.mean(d * d, axis=-1, keepdims=True)
    return d, lax.rsqrt(v + 1e-5) * scale


S3, S4 = 3, 2


def kern(u_h, are_h, aim_h, bre_h, bim_h, cre_h, cim_h, ldt, dsk, w1_h, w2_h, w3_h, w4_h, fwd_h, inv_h, fk_h, o_h,
         u, par, w1, w2, w3, w4, fwd, inv, fk, o_s, sems, isem, osem,
         dts, kt, kf, xf, xn_s, wr_s, h_s, g_s, z_s, dk_s, x1_s, xa_s):
    def in_copies(i):
        ps = pl.ds(pl.multiple_of(i * 64, 64), 64)
        xs = pl.ds(pl.multiple_of(i * 256, 256), 256)
        cs = [pltpu.make_async_copy(h.at[ps], par.at[k, ps], isem.at[i])
              for k, h in enumerate((are_h, aim_h, bre_h, bim_h, cre_h, cim_h))]
        return cs + [pltpu.make_async_copy(u_h.at[xs], u.at[xs], isem.at[i])]
    wc = [pltpu.make_async_copy(h, v, sems.at[k]) for k, (h, v) in enumerate(
        ((w1_h, w1), (fwd_h, fwd), (fk_h, fk), (w2_h, w2), (w3_h, w3), (w4_h, w4), (inv_h, inv)))]
    for c in in_copies(0):
        c.start()
    wc[0].start(); wc[1].start(); wc[3].start()
    for c in in_copies(1):
        c.start()

    dt = jnp.exp(ldt[...].astype(F32)).astype(BF).astype(F32).reshape(1, D)
    for g in range(4):
        dts[g*128:(g+1)*128] = jnp.broadcast_to(dt[:, g*128:(g+1)*128], (128, 128)).T
    row = lax.broadcasted_iota(jnp.int32, (8, 128), 0)
    lane = lax.broadcasted_iota(jnp.int32, (8, 128), 1)
    lo = row < 4
    ev = (row & 1) == 0
    rev = lambda z: csel(ev, *[tuple(pltpu.roll(v, sh, 0) for v in z) for sh in (5, 7)])
    swp = lambda z: tuple(pltpu.roll(v, 4, 0) for v in z)
    h_s[:, 0:8] = jnp.zeros((4, 8, 128), F32)
    h_s[:, L+8:L+16] = jnp.zeros((4, 8, 128), F32)

    def kgen(r0, q0):
        sl = pl.ds(r0, 16)
        are, aim, bre, bim, cre, cim = [par[k, sl].astype(F32) for k in range(6)]
        d = dts[sl]
        e = jnp.exp(d * are)
        th = d * aim
        l1 = (e * jnp.cos(th), e * jnp.sin(th))
        l2 = csq(l1)
        c = cmul((cre, cim), (bre, bim))
        W = (c[0] * d, c[1] * d)
        wr_s[sl] = W[0].astype(BF)
        outs = [[] for _ in range(6)]
        for hh in range(2):
            hf = lambda v: (v[0][hh*8:hh*8+8], v[1][hh*8:hh*8+8])
            p1, p2, w = hf(l1), hf(l2), hf(W)
            r1, r2, rw = swp(p1), swp(p2), swp(w)
            accs = []
            for s in range(2):
                mix = (lambda a, b: csel(lo, a, b))
                a0 = mix(p1, r2) if s == 0 else mix(r1, p2)
                u2 = mix(p2, r2) if s == 0 else mix(r2, p2)
                wd = mix(w, rw) if s == 0 else mix(rw, w)
                a = [a0]
                for _ in range(8):
                    a.append(csq(a[-1]))
                lhs, rhs = build(a, u2, wd, mix, rev, swp, lo)
                P = dot_nt(lhs[0], rhs[0]) - dot_nt(lhs[1], rhs[1])
                for (a0i, n) in ((0, 4), (4, 4), (8, 2)):
                    acc = None
                    for i in range(n):
                        v = pltpu.roll(P[(a0i+i)*8:(a0i+i)*8+8], i, 1, stride=1, stride_axis=0)
                        acc = v if acc is None else jnp.where((lane & 3) == ((i + 3) & 3), v, acc)
                    accs.append(acc)
            for t in range(3):
                outs[2*t].append(jnp.where(lo, accs[t], pltpu.roll(accs[3+t], 4, 0)))
                outs[2*t+1].append(jnp.where(lo, pltpu.roll(accs[t], 4, 0), accs[3+t]))
        for t in range(6):
            kt[t, sl] = jnp.concatenate(outs[t], 0).astype(BF)

    def pha(i):
        sl = pl.ds(pl.multiple_of(i * 256, 256), 256)
        d, r = ln_s(u[sl].astype(F32), 1.0)
        xn = d * r
        xn_s[sl] = xn
        XB = xn.astype(BF)
        yield
        xb = XB
        h = gelu_s(dot(xb, w1[...]) * GS) * GO
        for k in range(4):
            h_s[k, pl.ds(pl.multiple_of(i * 256 + 8, 8), 256)] = h[:, k*128:(k+1)*128]
        for c in range(2):
            yield
            X = dot(fwd[...], XB[c*128:(c+1)*128])
            for g in range(4):
                a, b = X[0:128, g*128:(g+1)*128], X[128:256, g*128:(g+1)*128]
                xf[g, 2*i + c, 0:128] = a + b
                xf[g, 2*i + c, 128:256] = a
                xf[g, 2*i + c, 256:384] = b

    def tok2(i):
        sl = pl.ds(pl.multiple_of(i * 256, 256), 256)
        b = i * 256 + 8
        hs = jnp.concatenate([h_s[k, pl.ds(b - sh, 256)] for k, sh in enumerate((1, -1, 2, -2))], 1).astype(BF)
        x1 = xn_s[sl] + dot(hs, w2[...])
        d, r = ln_s(x1, GS)
        x1_s[sl] = x1
        xa_s[sl] = (d * r).astype(BF)

    def pa(i, _, t):
        for c in in_copies(i):
            c.wait()
        @pl.when(i == 0)
        def _():
            wc[0].wait(); wc[1].wait()
        @pl.when(i + 2 < 8)
        def _():
            for c in in_copies(i + 2):
                c.start()
        for k in (2, 4, 5, 6):
            @pl.when(i == (0 if k == 2 else k - 3))
            def _():
                wc[k].start()
        gen = pha(i)
        next(gen, None)
        j = 0
        for ch in 'tkpkkpkp':
            if ch == 'k':
                kgen(pl.multiple_of(i * 64 + j * 16, 16), 0)
                j += 1
            elif ch == 'p':
                next(gen, None)
            elif t:
                tok2(i - 2)
        return 0
    with jax.named_scope('pa'):
        lax.fori_loop(0, 2, lambda i, c: pa(i, c, 0), 0)
        wc[3].wait()
        lax.fori_loop(2, 8, lambda i, c: pa(i, c, 1), 0)

    ones = jnp.ones((8, 128), BF)
    lane2 = lax.broadcasted_iota(jnp.int32, (128, 128), 1)
    for g in range(4):
        gs = slice(g*128, (g+1)*128)
        dk_s[:, gs] = dot_nt(ones, wr_s[gs]) + dsk[...].astype(F32).reshape(1, D)[:, gs]
    wc[2].wait()

    def kdft(g, _):
        gs = pl.ds(pl.multiple_of(g * 128, 128), 128)
        T = [kt[t, gs] for t in range(6)]
        for m in range(16):
            r = None
            for p, (m2, t, t2) in enumerate(PIECES):
                if m2 != m:
                    continue
                w = T[t]
                if t2 is not None:
                    w = jnp.where(lane2 == t2[1], pltpu.bitcast(pltpu.roll(pltpu.bitcast(T[t2[0]], jnp.int32), 124, 1), BF), w)
                v = dot_nt(fk[p], w)
                r = v if r is None else r + v
            c, d = r[0:128], r[128:256]
            kf[g, m, 0:128] = c
            kf[g, m, 128:256] = d - c
            kf[g, m, 256:384] = c + d
        return 0
    with jax.named_scope('kdft'):
        lax.fori_loop(0, 4, kdft, 0)

    def pw(i, par_, g):
        o = i * 8 + par_ * 64
        ld = lambda ref, m: tuple(ref[g, m, pl.ds(pl.multiple_of(o + k * 128, 8), 8)] for k in range(3))
        prev = None
        BL = 4
        for c0 in range(0, 16, BL):
            acc = [None] * BL
            Xc = {}
            for m in range(c0 + BL):
                yield
                K = ld(kf, m)
                for j in range(BL):
                    n = c0 + j - m
                    if n < 0:
                        continue
                    if n not in Xc:
                        Xc[n] = ld(xf, n)
                    t = tuple(K[k] * Xc[n][k] for k in range(3))
                    acc[j] = t if acc[j] is None else tuple(x + y for x, y in zip(acc[j], t))
            for j in range(BL):
                z = (acc[j][0] - acc[j][2], acc[j][0] + acc[j][1])
                zz = z
                if prev is not None:
                    zz = (z[0] - prev[1], z[1] + prev[0]) if par_ == 0 else (z[0] + prev[1], z[1] - prev[0])
                prev = z
                z_s[c0 + j, g, pl.ds(pl.multiple_of(i * 32 + par_ * 16, 16), 16)] = jnp.concatenate(zz, 0).astype(BF)

    wc[4].wait(); wc[5].wait(); wc[6].wait()

    def allpw(i):
        for j in range(8):
            yield from pw(i, j % 2, j // 2)

    def gate(i, v, steps):
        if gate.g is None:
            return
        for r in range(32, 257, 32):
            kf[pl.ds(jnp.minimum(i + 4, 4), 1), 0, 0:8, 0:min(128, v.shape[1])] = v[r-8:r][None]
            for _ in range(steps):
                next(gate.g, None)

    tok2(6)
    tok2(7)

    def phb(i, _):
        gate.g = allpw(i)
        sl = pl.ds(pl.multiple_of(i * 256, 256), 256)
        xa = xa_s[sl]
        hs = []
        for n0 in range(0, F, 128):
            v = dot_nt(xa, w3[n0:min(n0 + 128, F)])
            nv = v.shape[1]
            gate(i, v, S3)
            hs.append(gelu_s(v).astype(BF))
        h2 = jnp.concatenate(hs, 1)
        v4 = dot(h2, w4[...])
        for n in range(4):
            ns = slice(n * 128, n * 128 + 128)
            v = v4[:, ns]
            gate(i, v, S4)
            r = x1_s[sl, ns] + v * GO
            g_s[sl, ns] = r * jax.nn.sigmoid(r)
        for _ in gate.g:
            pass
        return 0
    with jax.named_scope('phb'):
        lax.fori_loop(0, 8, phb, 0)

    def out_copy(c):
        sl = pl.ds(pl.multiple_of(c * 256, 256), 256)
        return pltpu.make_async_copy(o_s.at[sl], o_h.at[sl], osem.at[c])

    def phc(c, _):
        for j in range(2):
            sl = pl.ds(pl.multiple_of(c * 256 + j * 128, 128), 128)
            for g in range(4):
                gs = slice(g*128, (g+1)*128)
                y = dot(inv[...], z_s[2*c + j, g]) + xn_s[sl, gs] * dk_s[0:1, gs]
                o_s[sl, gs] = (u[sl, gs].astype(F32) + y * g_s[sl, gs]).astype(BF)
        out_copy(c).start()
        return 0
    with jax.named_scope('phc'):
        lax.fori_loop(0, 8, phc, 0)
    for c in range(8):
        out_copy(c).wait()


def build(a, u2, wd, mix, rev, swp, lo):
    u4 = csq(u2)
    u8 = csq(u4)
    u256 = mix(a[8], swp(a[7]))
    ta = [cmul(wd, a[0])]
    for _ in range(3):
        ta.append(cmul(ta[-1], u2))
    t0 = cmul(cmul(wd, a[1]), a[8])
    t2 = cmul(t0, mix(u4, u256))
    tb = [t0, cmul(t0, a[1]), t2, cmul(t2, a[1])]
    u1024 = csq(csq(u256))
    w8 = cmul(cmul(wd, u8), u1024)
    tc0 = cmul(w8, (jnp.where(lo, 1.0, a[8][0]), jnp.where(lo, 0.0, a[8][1])))
    lhs = ta + tb + [tc0, cmul(tc0, u256)]
    l8 = rev(u8)
    l16 = csq(l8)
    rhs = [(jnp.where(lo, 1.0, l8[0]), jnp.where(lo, 0.0, l8[1]))]
    for _ in range(15):
        rhs.append(cmul(rhs[-1], l16))
    cat = lambda v: tuple(jnp.concatenate([x[k] for x in v], 0).astype(BF) for k in range(2))
    return cat(lhs), cat(rhs)


@jax.jit
def pallas_recurrent_scan__ssm_conv_s4__mixer_s_mlp__prompt_kernel(A_u, A_A_re, A_A_im, A_B_re, A_B_im, A_C_re, A_C_im, A_log_dt, A_Dskip, B_x, B_w1, B_w2, B_w3, B_w4):
    perm = np.arange(256).reshape(2, 2, 8, 8).transpose(2, 1, 0, 3).reshape(-1)
    hbm = pl.BlockSpec(memory_space=pltpu.HBM)
    vm = pl.BlockSpec(memory_space=pltpu.VMEM)
    V = pltpu.VMEM
    out = pl.pallas_call(
        kern,
        out_shape=jax.ShapeDtypeStruct((L, D), BF),
        grid=(1,),
        in_specs=[hbm] * 7 + [vm, vm] + [hbm] * 7,
        out_specs=hbm,
        scratch_shapes=[
            V((L, D), BF), V((6, D + 16, N), BF), V((D, D), BF), V((D, D), BF), V((F, D), BF), V((F, D), BF),
            V((256, 128), BF), V((128, 256), BF), V((18, 256, 128), BF), V((L, D), BF),
            pltpu.SemaphoreType.DMA((7,)), pltpu.SemaphoreType.DMA((8,)), pltpu.SemaphoreType.DMA((8,)),
            V((D, 128), F32), V((6, D, 128), BF), V((5, 16, 384, 128), F32),
            V((4, 16, 384, 128), F32), V((L, D), F32), V((D, 128), BF),
            V((4, L + 16, 128), F32), V((L, D), F32), V((16, 4, 256, 128), BF),
            V((8, D), F32), V((L, D), F32), V((L, D), BF)],
        compiler_params=pltpu.CompilerParams(vmem_limit_bytes=110 * 2**20),
    )(A_u.reshape(L, D), A_A_re, A_A_im, A_B_re, A_B_im, A_C_re, A_C_im, A_log_dt,
      A_Dskip, B_w1, B_w2, B_w3.T, B_w4, FWD, INV[:, perm], FK)
    return out.reshape(1, L, D)
```
